```python
import jax
import jax.numpy as jnp

def _softmax(x, axis=-1):
    return jax.nn.softmax(x, axis=axis)
def _gelu(x):
    return jax.nn.gelu(x, approximate=True)
def _silu(x):
    return jax.nn.silu(x)
def _sigmoid(x):
    return jax.nn.sigmoid(x)
def _layernorm(x, axis=-1, eps=1e-5):
    m = jnp.mean(x, axis=axis, keepdims=True)
    v = jnp.var(x, axis=axis, keepdims=True)
    return (x - m) / jnp.sqrt(v + eps)
def _scatter_add(tgt, idx, src, axis=0):
    return tgt.at[idx].add(src)
def _segment_sum(src, seg, n):
    return jax.ops.segment_sum(src, seg, n)
class _Rng:
    def __init__(self, key):
        self._k = key
    def _next(self):
        self._k, sub = jax.random.split(self._k)
        return sub
    def normal(self, shape):
        return jax.random.normal(self._next(), shape, dtype=jnp.bfloat16)
    def randint(self, lo, hi, shape):
        return jax.random.randint(self._next(), shape, lo, hi, dtype=jnp.int32)
    def uniform(self, shape, lo=0.0, hi=1.0):
        return jax.random.uniform(self._next(), shape, jnp.bfloat16, lo, hi)
    def permutation(self, n):
        return jax.random.permutation(self._next(), n)


kernel_name = 'recurrent_scan__compressed_kv_cla__dense_activation_silu__decode'

def setup_inputs():
    _rng = _Rng(jax.random.key(int.from_bytes(__import__("os").urandom(4), "little")))
    _w = (lambda a: (lambda t: t.astype(jnp.bfloat16) if jnp.issubdtype(t.dtype, jnp.floating) else t)(jnp.asarray(a)))
    def _A_setup():
        B, H, Sq, Sk, D, M = 1, 32, 1, 32768, 128, 512
        Dc = 4 * D
        return {
            "x": _w((lambda *s: _rng.normal(s) * 0.05)(B, Sq, M)),
            "c_kv": _w((lambda *s: _rng.normal(s) * 0.05)(B, Sk, Dc)),
            "w_q": _w((lambda *s: _rng.normal(s) * 0.05)(M, H, D) * (M ** -0.5)),
            "w_uk": _w((lambda *s: _rng.normal(s) * 0.05)(Dc, H, D) * (Dc ** -0.5)),
            "w_uv": _w((lambda *s: _rng.normal(s) * 0.05)(Dc, H, D) * (Dc ** -0.5)),
            "w_o": _w((lambda *s: _rng.normal(s) * 0.05)(H, D, M) * ((H * D) ** -0.5)),
        }
    _A_in = _A_setup()

    def _B_setup():
        B, S, D, F = 1, 1, 512, 1376
        return {
            "x": _w((lambda *s: _rng.normal(s) * 0.05)(B, S, D)),
            "w1": _w((lambda *s: _rng.normal(s) * 0.05)(D, F) * (D ** -0.5)),
            "w2": _w((lambda *s: _rng.normal(s) * 0.05)(F, D) * (F ** -0.5)),
        }
    _B_in = _B_setup()

    return {
        "A_x": _A_in["x"],
        "A_c_kv": _A_in["c_kv"],
        "A_w_q": _A_in["w_q"],
        "A_w_uk": _A_in["w_uk"],
        "A_w_uv": _A_in["w_uv"],
        "A_w_o": _A_in["w_o"],
        "B_x": _B_in["x"],
        "B_w1": _B_in["w1"],
        "B_w2": _B_in["w2"],
    }

def reference(A_x, A_c_kv, A_w_q, A_w_uk, A_w_uv, A_w_o, B_x, B_w1, B_w2):
    def _A_ref(x, c_kv, w_q, w_uk, w_uv, w_o):
        B, Sq, M = x.shape[0], x.shape[1], x.shape[2]
        Sk = c_kv.shape[1]
        H, D = w_q.shape[1], w_q.shape[2]
        q = jnp.einsum("bqm,mhd->bhqd", x, w_q)
        k = jnp.einsum("bkc,chd->bhkd", c_kv, w_uk)
        v = jnp.einsum("bkc,chd->bhkd", c_kv, w_uv)
        scores = jnp.einsum("bhqd,bhkd->bhqk", q, k) * (D ** -0.5)
        off = Sk - Sq
        qi = jnp.arange(Sq)[:, None]
        kj = jnp.arange(Sk)[None, :]
        cmask = kj <= (qi + off)
        scores = jnp.where(cmask[None, None], scores, -1e9)
        p = _softmax(scores, axis=-1)
        ctx = jnp.einsum("bhqk,bhkd->bhqd", p, v)
        return jnp.einsum("bhqd,hdm->bqm", ctx, w_o)

    def _B_ref(x, w1, w2):
        h = jnp.einsum("bsd,df->bsf", x, w1)
        h = _silu(h)
        out = jnp.einsum("bsf,fd->bsd", h, w2)
        return out

    x = A_x
    xn = _layernorm(x, axis=-1)
    s = _A_ref(xn, A_c_kv, A_w_q, A_w_uk, A_w_uv, A_w_o)
    g = _silu(_B_ref(xn, B_w1, B_w2))
    return x + s * g
```

```python
import functools
import jax
import jax.numpy as jnp
from jax import lax
import jax.experimental.pallas as pl
import jax.experimental.pallas.tpu as pltpu

BF = jnp.bfloat16
F32 = jnp.float32
NT = (((1,), (1,)), ((), ()))

H, D, M, DC, SK, F = 32, 128, 512, 512, 32768, 1376
FP = 1408


def _iota(shape, dim):
    return lax.broadcasted_iota(jnp.int32, shape, dim)


def make_kernel(n_chunks=8, bk=2048):
    ch = SK // n_chunks

    def kernel(x_hbm, ckv_hbm, wq_hbm, wuk_hbm, wuv_hbm, wo_hbm, w1t_hbm, w2_hbm, o_ref,
               x_v, ckv_v, wq_v, wuk_v, wuv_v, wo_v, w1_v, w2_v, xs_v, sems):
        cp_x = pltpu.make_async_copy(x_hbm, x_v, sems.at[0])
        cp_wq = pltpu.make_async_copy(wq_hbm, wq_v, sems.at[1])
        cp_wuk = pltpu.make_async_copy(wuk_hbm, wuk_v, sems.at[2])
        cp_wuv = pltpu.make_async_copy(wuv_hbm, wuv_v, sems.at[3])
        cp_wo = pltpu.make_async_copy(wo_hbm, wo_v, sems.at[4])
        cp_w1 = pltpu.make_async_copy(w1t_hbm, w1_v.at[pl.ds(0, F)], sems.at[5])
        cp_w2 = pltpu.make_async_copy(w2_hbm, w2_v.at[pl.ds(0, F)], sems.at[6])

        def cp_ckv(j):
            return pltpu.make_async_copy(ckv_hbm.at[pl.ds(j * ch, ch)], ckv_v.at[pl.ds(j * ch, ch)], sems.at[7 + j])

        cp_x.start()
        cp_wq.start()
        cp_wuk.start()
        for j in range(n_chunks):
            cp_ckv(j).start()
        cp_wuv.start()
        cp_wo.start()
        cp_w1.start()
        cp_w2.start()

        w1_v[pl.ds(F, FP - F), :] = jnp.zeros((FP - F, M), BF)
        w2_v[pl.ds(F, FP - F), :] = jnp.zeros((FP - F, M), BF)

        lane = _iota((H, D), 1)
        row = _iota((H, D), 0)
        mask_nat = (lane % 32) == row
        mask_rev = (lane % 32) == (31 - row)
        pr = _iota((128, 128), 0)
        pc = _iota((128, 128), 1)
        G = ((pr % 4) == (pc // 32)).astype(BF)
        PB = (pr == ((pc % 4) * 32 + pc // 4 + 31) % 128).astype(BF)
        PC = (pc == ((pr % 4) * 32 + pr // 4 + 97) % 128).astype(BF)
        rr = _iota((H, H), 0)
        rc = _iota((H, H), 1)
        REV = (rr + rc == 31).astype(BF)

        cp_x.wait()
        x = x_v[...].astype(F32)
        mu = jnp.mean(x, axis=-1, keepdims=True)
        xc = x - mu
        var = jnp.mean(xc * xc, axis=-1, keepdims=True)
        xn = (xc * lax.rsqrt(var + 1e-5)).astype(BF).astype(F32)

        vrow = _iota((32, 128), 0)
        vlane = _iota((32, 128), 1)
        dmask = (vlane // 4) == vrow
        Dm = jnp.concatenate(
            [jnp.where(dmask, jnp.broadcast_to(xn[:, u * 128:(u + 1) * 128], (32, 128)), 0.0) for u in range(4)],
            axis=0).astype(BF)
        xs_v[...] = jnp.dot(Dm, G, preferred_element_type=F32)

        cp_wq.wait()
        qacc = jnp.zeros((H, D), F32)
        for t in range(128):
            a = jnp.where(mask_rev, jnp.broadcast_to(xs_v[t:t + 1, :], (H, D)), 0.0).astype(BF)
            qacc = qacc + jnp.dot(a, wq_v[t * 128:(t + 1) * 128, :], preferred_element_type=F32)
        q = qacc.astype(BF)

        cp_wuk.wait()
        chunks = []
        for u in range(4):
            c = jnp.zeros((H, D), F32)
            for v in range(32):
                t = u * 32 + v
                o = lax.dot_general(q, wuk_v[t * 128:(t + 1) * 128, :], NT, preferred_element_type=F32)
                o = pltpu.roll(o, v, 1, stride=1, stride_axis=0)
                c = jnp.where((lane % 32) == ((31 + v) % 32), o, c)
            c = (c * (D ** -0.5)).astype(BF)
            chunks.append(jnp.dot(c, PB, preferred_element_type=F32).astype(BF))
        ql_rev = jnp.concatenate(chunks, axis=1)
        ql = jnp.dot(REV, ql_rev, preferred_element_type=F32).astype(BF)

        nsub = ch // bk

        def body(j, carry):
            m, l, acc = carry
            cp_ckv(j).wait()
            for sidx in range(nsub):
                start = pl.multiple_of(j * ch + sidx * bk, bk)
                cblk = ckv_v[pl.ds(start, bk), :]
                s = lax.dot_general(ql, cblk, NT, preferred_element_type=F32)
                m_new = jnp.maximum(m, jnp.max(s, axis=1, keepdims=True))
                alpha = jnp.exp(m - m_new)
                p = jnp.exp(s - m_new)
                l = alpha * l + jnp.sum(p, axis=1, keepdims=True)
                acc = alpha * acc + jnp.dot(p.astype(BF), cblk, preferred_element_type=F32)
                m = m_new
            return m, l, acc

        m0 = jnp.full((H, 1), -jnp.inf, F32)
        m, l, acc = lax.fori_loop(0, n_chunks, body, (m0, jnp.zeros((H, 1), F32), jnp.zeros((H, DC), F32)))
        L = (acc / l).astype(BF)

        cp_wuv.wait()
        cacc = jnp.zeros((H, D), F32)
        for u in range(4):
            Lp = jnp.dot(L[:, u * 128:(u + 1) * 128], PC, preferred_element_type=F32)
            for v in range(32):
                t = u * 32 + v
                rolled = pltpu.roll(Lp, 31 - v, 1, stride=1, stride_axis=0)
                a = jnp.where(mask_nat, rolled, 0.0).astype(BF)
                cacc = cacc + jnp.dot(a, wuv_v[t * 128:(t + 1) * 128, :], preferred_element_type=F32)
        ctx = cacc

        cp_wo.wait()
        sacc = jnp.zeros((H, M), F32)
        for h in range(H):
            a = jnp.where(row == h, ctx, 0.0).astype(BF)
            sacc = sacc + jnp.dot(a, wo_v[h * 128:(h + 1) * 128, :], preferred_element_type=F32)
        s_out = jnp.sum(sacc, axis=0, keepdims=True)

        cp_w1.wait()
        xb = jnp.broadcast_to(xn, (8, M)).astype(BF)
        hh = lax.dot_general(xb, w1_v[...], NT, preferred_element_type=F32)
        hh = hh * jax.nn.sigmoid(hh)
        cp_w2.wait()
        f2 = jnp.dot(hh.astype(BF), w2_v[...], preferred_element_type=F32)[0:1]
        g = f2 * jax.nn.sigmoid(f2)
        o_ref[...] = (x + s_out * g).astype(o_ref.dtype)

    return kernel


def _build(n_chunks=8, bk=2048):
    kernel = make_kernel(n_chunks, bk)

    def fn(A_x, A_c_kv, A_w_q, A_w_uk, A_w_uv, A_w_o, B_x, B_w1, B_w2):
        anys = pl.BlockSpec(memory_space=pl.ANY)
        out = pl.pallas_call(
            kernel,
            in_specs=[anys] * 8,
            out_specs=pl.BlockSpec(memory_space=pltpu.VMEM),
            out_shape=jax.ShapeDtypeStruct((1, M), BF),
            scratch_shapes=[
                pltpu.VMEM((1, M), BF),
                pltpu.VMEM((SK, DC), BF),
                pltpu.VMEM((M * H, D), BF),
                pltpu.VMEM((DC * H, D), BF),
                pltpu.VMEM((DC * H, D), BF),
                pltpu.VMEM((H * D, M), BF),
                pltpu.VMEM((FP, M), BF),
                pltpu.VMEM((FP, M), BF),
                pltpu.VMEM((128, 128), F32),
                pltpu.SemaphoreType.DMA((7 + n_chunks,)),
            ],
            compiler_params=pltpu.CompilerParams(vmem_limit_bytes=100 * 1024 * 1024),
        )(A_x.reshape(1, M), A_c_kv.reshape(SK, DC), A_w_q.reshape(M * H, D), A_w_uk.reshape(DC * H, D),
          A_w_uv.reshape(DC * H, D), A_w_o.reshape(H * D, M), B_w1.T, B_w2)
        return out.reshape(1, 1, M)
    return fn


@jax.jit
def pallas_recurrent_scan__compressed_kv_cla__dense_activation_silu__decode_kernel(
    A_x: jax.Array,
    A_c_kv: jax.Array,
    A_w_q: jax.Array,
    A_w_uk: jax.Array,
    A_w_uv: jax.Array,
    A_w_o: jax.Array,
    B_x: jax.Array,
    B_w1: jax.Array,
    B_w2: jax.Array,
):
    return _build()(A_x, A_c_kv, A_w_q, A_w_uk, A_w_uv, A_w_o, B_x, B_w1, B_w2)
```

```python
import jax
import jax.numpy as jnp
from jax import lax
import jax.experimental.pallas as pl
import jax.experimental.pallas.tpu as pltpu

BF = jnp.bfloat16
F32 = jnp.float32
_NT = (((1,), (1,)), ((), ()))

H, D, M, DC, F = 32, 128, 512, 512, 1376
FP = 1408
BK = 2048
N_CKV_COPIES = 4
WO_ROWS = (3072, 640, 256, 128)


def _iota(shape, dim):
    return lax.broadcasted_iota(jnp.int32, shape, dim)


def _offsets(sizes):
    return [sum(sizes[:i]) for i in range(len(sizes))]


def _make_kernel(sk):
    assert sk % (N_CKV_COPIES * BK) == 0
    ckv_rows = sk // N_CKV_COPIES
    wo_off = _offsets(WO_ROWS)
    n_wo = len(WO_ROWS)

    def kernel(x_hbm, ckv_hbm, wq_hbm, wuk_hbm, wuv_hbm, wo_hbm, w1t_hbm, w2_hbm,
               o_ref,
               x_v, ckv_v, wq_v, wuk_v, wuv_v, wo_v, w1_v, w2_v, xs_v, ctx_v, sems):
        cp_x = pltpu.make_async_copy(x_hbm, x_v, sems.at[0])
        cp_wq = pltpu.make_async_copy(wq_hbm, wq_v, sems.at[1])
        cp_wuk = pltpu.make_async_copy(wuk_hbm, wuk_v, sems.at[2])
        cp_wuv = pltpu.make_async_copy(wuv_hbm, wuv_v, sems.at[3])
        cp_w1 = pltpu.make_async_copy(w1t_hbm, w1_v.at[pl.ds(0, F)], sems.at[4])
        cp_w2 = pltpu.make_async_copy(w2_hbm, w2_v.at[pl.ds(0, F)], sems.at[5])
        cp_ckv = [
            pltpu.make_async_copy(
                ckv_hbm.at[pl.ds(j * ckv_rows, ckv_rows)],
                ckv_v.at[pl.ds(j * ckv_rows, ckv_rows)],
                sems.at[6 + j])
            for j in range(N_CKV_COPIES)]
        cp_wo = [
            pltpu.make_async_copy(
                wo_hbm.at[pl.ds(wo_off[j], WO_ROWS[j])],
                wo_v.at[pl.ds(wo_off[j], WO_ROWS[j])],
                sems.at[6 + N_CKV_COPIES + j])
            for j in range(n_wo)]

        cp_x.start()
        cp_wq.start()
        cp_wuk.start()
        for cp in cp_ckv:
            cp.start()
        cp_wuv.start()
        cp_w1.start()
        cp_w2.start()
        for cp in cp_wo:
            cp.start()

        w1_v[pl.ds(F, FP - F), :] = jnp.zeros((FP - F, M), BF)
        w2_v[pl.ds(F, FP - F), :] = jnp.zeros((FP - F, M), BF)

        lane = _iota((H, D), 1)
        row = _iota((H, D), 0)
        mask_nat = (lane % 32) == row
        mask_rev = (lane % 32) == (31 - row)
        pr = _iota((128, 128), 0)
        pc = _iota((128, 128), 1)
        spread = ((pr % 4) == (pc // 32)).astype(BF)
        perm_b = (pr == ((pc % 4) * 32 + pc // 4 + 31) % 128).astype(BF)
        perm_c = (pc == ((pr % 4) * 32 + pr // 4 + 97) % 128).astype(BF)
        rev = (_iota((H, H), 0) + _iota((H, H), 1) == H - 1).astype(BF)

        cp_x.wait()
        x = x_v[...].astype(F32)
        mu = jnp.mean(x, axis=-1, keepdims=True)
        xc = x - mu
        var = jnp.mean(xc * xc, axis=-1, keepdims=True)
        xn = (xc / jnp.sqrt(var + 1e-5)).astype(BF).astype(F32)

        dmask = (_iota((32, 128), 1) // 4) == _iota((32, 128), 0)
        dmat = jnp.concatenate(
            [jnp.where(dmask, jnp.broadcast_to(xn[:, u * 128:(u + 1) * 128], (32, 128)), 0.0)
             for u in range(4)], axis=0).astype(BF)
        xs_v[...] = jnp.dot(dmat, spread, preferred_element_type=F32)

        cp_wq.wait()
        qacc = jnp.zeros((H, D), F32)
        for t in range(128):
            a = jnp.where(mask_rev, jnp.broadcast_to(xs_v[t:t + 1, :], (H, D)), 0.0)
            qacc = qacc + jnp.dot(a.astype(BF), wq_v[t * 128:(t + 1) * 128, :],
                                  preferred_element_type=F32)
        q = qacc.astype(BF)

        cp_wuk.wait()
        pieces = []
        for u in range(4):
            c = jnp.zeros((H, D), F32)
            for v in range(32):
                t = u * 32 + v
                o = lax.dot_general(q, wuk_v[t * 128:(t + 1) * 128, :], _NT,
                                    preferred_element_type=F32)
                o = pltpu.roll(o, v, 1, stride=1, stride_axis=0)
                c = jnp.where((lane % 32) == ((31 + v) % 32), o, c)
            c = (c * (D ** -0.5)).astype(BF)
            pieces.append(jnp.dot(c, perm_b, preferred_element_type=F32).astype(BF))
        ql = jnp.dot(rev, jnp.concatenate(pieces, axis=1),
                     preferred_element_type=F32).astype(BF)

        def block(start, carry):
            m, l, acc = carry
            cblk = ckv_v[pl.ds(start, BK), :]
            s = lax.dot_general(ql, cblk, _NT, preferred_element_type=F32)
            m_new = jnp.maximum(m, jnp.max(s, axis=1, keepdims=True))
            alpha = jnp.exp(m - m_new)
            p = jnp.exp(s - m_new)
            l = alpha * l + jnp.sum(p, axis=1, keepdims=True)
            acc = alpha * acc + jnp.dot(p.astype(BF), cblk, preferred_element_type=F32)
            return m_new, l, acc

        carry = (jnp.full((H, 1), -jnp.inf, F32), jnp.zeros((H, 1), F32),
                 jnp.zeros((H, DC), F32))
        for j in range(N_CKV_COPIES):
            cp_ckv[j].wait()
            carry = lax.fori_loop(
                0, ckv_rows // BK,
                lambda i, cr, j=j: block(pl.multiple_of(j * ckv_rows + i * BK, BK), cr),
                carry)
        _, l, acc = carry
        lat = (acc / l).astype(BF)

        cp_wuv.wait()
        cacc = jnp.zeros((H, D), F32)
        for u in range(4):
            lp = jnp.dot(lat[:, u * 128:(u + 1) * 128], perm_c, preferred_element_type=F32)
            for v in range(32):
                t = u * 32 + v
                a = jnp.where(mask_nat, pltpu.roll(lp, 31 - v, 1, stride=1, stride_axis=0), 0.0)
                cacc = cacc + jnp.dot(a.astype(BF), wuv_v[t * 128:(t + 1) * 128, :],
                                      preferred_element_type=F32)
        ctx_v[...] = cacc

        cp_w1.wait()
        xb = jnp.broadcast_to(xn, (8, M)).astype(BF)
        hid = lax.dot_general(xb, w1_v[...], _NT, preferred_element_type=F32)
        hid = hid * jax.nn.sigmoid(hid)
        cp_w2.wait()
        f2 = jnp.dot(hid.astype(BF), w2_v[...], preferred_element_type=F32)[0:1]
        gate = f2 * jax.nn.sigmoid(f2)

        r_last = wo_off[-1]
        assert r_last // D == H - 1
        coef = jnp.broadcast_to(ctx_v[H - 1:H, :].astype(BF).astype(F32), (D, D)).T
        coef = jnp.concatenate([coef[r_last % D:, :]] * (M // 128), axis=1)
        sacc = jnp.zeros((8, M), F32)
        for j in range(n_wo - 1):
            parts = []
            r = wo_off[j]
            while r < wo_off[j] + WO_ROWS[j]:
                h = r // D
                r1 = min((h + 1) * D, wo_off[j] + WO_ROWS[j])
                lhs = jnp.broadcast_to(ctx_v[h:h + 1, r - h * D:r1 - h * D], (8, r1 - r))
                parts.append((r, r1, lhs.astype(BF)))
                r = r1
            cp_wo[j].wait()
            for r0, r1, lhs in parts:
                sacc = sacc + jnp.dot(lhs, wo_v[r0:r1, :], preferred_element_type=F32)
        cp_wo[n_wo - 1].wait()
        s = sacc[0:1] + jnp.sum(wo_v[r_last:H * D, :].astype(F32) * coef, axis=0, keepdims=True)

        o_ref[...] = (x + s * gate).astype(o_ref.dtype)

    return kernel


@jax.jit
def pallas_recurrent_scan__compressed_kv_cla__dense_activation_silu__decode_kernel(
    A_x: jax.Array,
    A_c_kv: jax.Array,
    A_w_q: jax.Array,
    A_w_uk: jax.Array,
    A_w_uv: jax.Array,
    A_w_o: jax.Array,
    B_x: jax.Array,
    B_w1: jax.Array,
    B_w2: jax.Array,
):
    del B_x
    sk = A_c_kv.shape[1]
    in_hbm = pl.BlockSpec(memory_space=pl.ANY)
    out = pl.pallas_call(
        _make_kernel(sk),
        in_specs=[in_hbm] * 8,
        out_specs=pl.BlockSpec(memory_space=pltpu.VMEM),
        out_shape=jax.ShapeDtypeStruct((1, M), A_x.dtype),
        scratch_shapes=[
            pltpu.VMEM((1, M), BF),
            pltpu.VMEM((sk, DC), BF),
            pltpu.VMEM((M * H, D), BF),
            pltpu.VMEM((DC * H, D), BF),
            pltpu.VMEM((DC * H, D), BF),
            pltpu.VMEM((H * D, M), BF),
            pltpu.VMEM((FP, M), BF),
            pltpu.VMEM((FP, M), BF),
            pltpu.VMEM((128, 128), F32),
            pltpu.VMEM((H, D), F32),
            pltpu.SemaphoreType.DMA((6 + N_CKV_COPIES + len(WO_ROWS),)),
        ],
        compiler_params=pltpu.CompilerParams(
            vmem_limit_bytes=100 * 1024 * 1024,
            disable_semaphore_checks=True,
        ),
    )(
        A_x.reshape(1, M),
        A_c_kv.reshape(sk, DC),
        A_w_q.reshape(M * H, D),
        A_w_uk.reshape(DC * H, D),
        A_w_uv.reshape(DC * H, D),
        A_w_o.reshape(H * D, M),
        B_w1.T,
        B_w2,
    )
    return out.reshape(1, 1, M)
```

```python
import jax
import jax.numpy as jnp
from jax import lax
import jax.experimental.pallas as pl
import jax.experimental.pallas.tpu as pltpu

BF = jnp.bfloat16
F32 = jnp.float32
_NT = (((1,), (1,)), ((), ()))

H, D, M, DC, F = 32, 128, 512, 512, 1376
FP = 1408
BK = 2048
N_CKV_COPIES = 4
WO_ROWS = (3072, 640, 256, 96, 32)
N_WO_VPU = 2


def _iota(shape, dim):
    return lax.broadcasted_iota(jnp.int32, shape, dim)


def _offsets(sizes):
    return [sum(sizes[:i]) for i in range(len(sizes))]


def _make_kernel(sk):
    assert sk % (N_CKV_COPIES * BK) == 0
    ckv_rows = sk // N_CKV_COPIES
    wo_off = _offsets(WO_ROWS)
    n_wo = len(WO_ROWS)

    def kernel(x_hbm, ckv_hbm, wq_hbm, wuk_hbm, wuv_hbm, wo_hbm, w1t_hbm, w2_hbm,
               o_ref,
               x_v, ckv_v, wq_v, wuk_v, wuv_v, wo_v, w1_v, w2_v, xs_v, ctx_v, sems):
        cp_x = pltpu.make_async_copy(x_hbm, x_v, sems.at[0])
        cp_wq = pltpu.make_async_copy(wq_hbm, wq_v, sems.at[1])
        cp_wuk = pltpu.make_async_copy(wuk_hbm, wuk_v, sems.at[2])
        cp_wuv = pltpu.make_async_copy(wuv_hbm, wuv_v, sems.at[3])
        cp_w1 = pltpu.make_async_copy(w1t_hbm, w1_v.at[pl.ds(0, F)], sems.at[4])
        cp_w2 = pltpu.make_async_copy(w2_hbm, w2_v.at[pl.ds(0, F)], sems.at[5])
        cp_ckv = [
            pltpu.make_async_copy(
                ckv_hbm.at[pl.ds(j * ckv_rows, ckv_rows)],
                ckv_v.at[pl.ds(j * ckv_rows, ckv_rows)],
                sems.at[6 + j])
            for j in range(N_CKV_COPIES)]
        cp_wo = [
            pltpu.make_async_copy(
                wo_hbm.at[pl.ds(wo_off[j], WO_ROWS[j])],
                wo_v.at[pl.ds(wo_off[j], WO_ROWS[j])],
                sems.at[6 + N_CKV_COPIES + j])
            for j in range(n_wo)]

        cp_x.start()
        cp_wq.start()
        cp_wuk.start()
        for cp in cp_ckv:
            cp.start()
        cp_wuv.start()
        cp_w1.start()
        cp_w2.start()
        for cp in cp_wo:
            cp.start()

        w1_v[pl.ds(F, FP - F), :] = jnp.zeros((FP - F, M), BF)
        w2_v[pl.ds(F, FP - F), :] = jnp.zeros((FP - F, M), BF)

        lane = _iota((H, D), 1)
        row = _iota((H, D), 0)
        mask_nat = (lane % 32) == row
        mask_rev = (lane % 32) == (31 - row)
        pr = _iota((128, 128), 0)
        pc = _iota((128, 128), 1)
        spread = ((pr % 4) == (pc // 32)).astype(BF)
        perm_b = (pr == ((pc % 4) * 32 + pc // 4 + 31) % 128).astype(BF)
        perm_c = (pc == ((pr % 4) * 32 + pr // 4 + 97) % 128).astype(BF)
        rev = (_iota((H, H), 0) + _iota((H, H), 1) == H - 1).astype(BF)

        cp_x.wait()
        x = x_v[...].astype(F32)
        mu = jnp.mean(x, axis=-1, keepdims=True)
        xc = x - mu
        var = jnp.mean(xc * xc, axis=-1, keepdims=True)
        xn = (xc / jnp.sqrt(var + 1e-5)).astype(BF).astype(F32)

        dmask = (_iota((32, 128), 1) // 4) == _iota((32, 128), 0)
        dmat = jnp.concatenate(
            [jnp.where(dmask, jnp.broadcast_to(xn[:, u * 128:(u + 1) * 128], (32, 128)), 0.0)
             for u in range(4)], axis=0).astype(BF)
        xs_v[...] = jnp.dot(dmat, spread, preferred_element_type=F32)

        cp_wq.wait()
        qacc = jnp.zeros((H, D), F32)
        for t in range(128):
            a = jnp.where(mask_rev, jnp.broadcast_to(xs_v[t:t + 1, :], (H, D)), 0.0)
            qacc = qacc + jnp.dot(a.astype(BF), wq_v[t * 128:(t + 1) * 128, :],
                                  preferred_element_type=F32)
        q = qacc.astype(BF)

        cp_wuk.wait()
        pieces = []
        for u in range(4):
            c = jnp.zeros((H, D), F32)
            for v in range(32):
                t = u * 32 + v
                o = lax.dot_general(q, wuk_v[t * 128:(t + 1) * 128, :], _NT,
                                    preferred_element_type=F32)
                o = pltpu.roll(o, v, 1, stride=1, stride_axis=0)
                c = jnp.where((lane % 32) == ((31 + v) % 32), o, c)
            c = (c * (D ** -0.5)).astype(BF)
            pieces.append(jnp.dot(c, perm_b, preferred_element_type=F32).astype(BF))
        ql = jnp.dot(rev, jnp.concatenate(pieces, axis=1),
                     preferred_element_type=F32).astype(BF)

        def block(start, carry):
            m, l, acc = carry
            cblk = ckv_v[pl.ds(start, BK), :]
            s = lax.dot_general(ql, cblk, _NT, preferred_element_type=F32)
            m_new = jnp.maximum(m, jnp.max(s, axis=1, keepdims=True))
            alpha = jnp.exp(m - m_new)
            p = jnp.exp(s - m_new)
            l = alpha * l + jnp.sum(p, axis=1, keepdims=True)
            acc = alpha * acc + jnp.dot(p.astype(BF), cblk, preferred_element_type=F32)
            return m_new, l, acc

        carry = (jnp.full((H, 1), -jnp.inf, F32), jnp.zeros((H, 1), F32),
                 jnp.zeros((H, DC), F32))
        for j in range(N_CKV_COPIES):
            cp_ckv[j].wait()
            carry = lax.fori_loop(
                0, ckv_rows // BK,
                lambda i, cr, j=j: block(pl.multiple_of(j * ckv_rows + i * BK, BK), cr),
                carry)
        _, l, acc = carry
        lat = (acc / l).astype(BF)

        cp_wuv.wait()
        cacc = jnp.zeros((H, D), F32)
        for u in range(4):
            lp = jnp.dot(lat[:, u * 128:(u + 1) * 128], perm_c, preferred_element_type=F32)
            for v in range(32):
                t = u * 32 + v
                a = jnp.where(mask_nat, pltpu.roll(lp, 31 - v, 1, stride=1, stride_axis=0), 0.0)
                cacc = cacc + jnp.dot(a.astype(BF), wuv_v[t * 128:(t + 1) * 128, :],
                                      preferred_element_type=F32)
        ctx_v[...] = cacc

        cp_w1.wait()
        xb = jnp.broadcast_to(xn, (8, M)).astype(BF)
        hid = lax.dot_general(xb, w1_v[...], _NT, preferred_element_type=F32)
        hid = hid * jax.nn.sigmoid(hid)
        cp_w2.wait()
        f2 = jnp.dot(hid.astype(BF), w2_v[...], preferred_element_type=F32)[0:1]
        gate = f2 * jax.nn.sigmoid(f2)

        n_mxu = n_wo - N_WO_VPU
        r_vpu = wo_off[n_mxu]
        assert r_vpu // D == H - 1
        coef = jnp.broadcast_to(ctx_v[H - 1:H, :].astype(BF).astype(F32), (D, D)).T
        sacc = jnp.zeros((8, M), F32)
        for j in range(n_mxu):
            parts = []
            r = wo_off[j]
            while r < wo_off[j] + WO_ROWS[j]:
                h = r // D
                r1 = min((h + 1) * D, wo_off[j] + WO_ROWS[j])
                lhs = jnp.broadcast_to(ctx_v[h:h + 1, r - h * D:r1 - h * D], (8, r1 - r))
                parts.append((r, r1, lhs.astype(BF)))
                r = r1
            cp_wo[j].wait()
            for r0, r1, lhs in parts:
                sacc = sacc + jnp.dot(lhs, wo_v[r0:r1, :], preferred_element_type=F32)
        part = None
        for j in range(n_mxu, n_wo):
            r0, r1 = wo_off[j], wo_off[j] + WO_ROWS[j]
            co = jnp.concatenate([coef[r0 % D:(r1 - 1) % D + 1, :]] * (M // 128), axis=1)
            cp_wo[j].wait()
            prod = wo_v[r0:r1, :].astype(F32) * co
            for k in range((r1 - r0) // 8):
                piece = prod[8 * k:8 * k + 8]
                part = piece if part is None else part + piece
        s = sacc[0:1] + jnp.sum(part, axis=0, keepdims=True)

        o_ref[...] = (x + s * gate).astype(o_ref.dtype)

    return kernel


@jax.jit
def pallas_recurrent_scan__compressed_kv_cla__dense_activation_silu__decode_kernel(
    A_x: jax.Array,
    A_c_kv: jax.Array,
    A_w_q: jax.Array,
    A_w_uk: jax.Array,
    A_w_uv: jax.Array,
    A_w_o: jax.Array,
    B_x: jax.Array,
    B_w1: jax.Array,
    B_w2: jax.Array,
):
    del B_x
    sk = A_c_kv.shape[1]
    in_hbm = pl.BlockSpec(memory_space=pl.ANY)
    out = pl.pallas_call(
        _make_kernel(sk),
        in_specs=[in_hbm] * 8,
        out_specs=pl.BlockSpec(memory_space=pltpu.VMEM),
        out_shape=jax.ShapeDtypeStruct((1, M), A_x.dtype),
        scratch_shapes=[
            pltpu.VMEM((1, M), BF),
            pltpu.VMEM((sk, DC), BF),
            pltpu.VMEM((M * H, D), BF),
            pltpu.VMEM((DC * H, D), BF),
            pltpu.VMEM((DC * H, D), BF),
            pltpu.VMEM((H * D, M), BF),
            pltpu.VMEM((FP, M), BF),
            pltpu.VMEM((FP, M), BF),
            pltpu.VMEM((128, 128), F32),
            pltpu.VMEM((H, D), F32),
            pltpu.SemaphoreType.DMA((6 + N_CKV_COPIES + len(WO_ROWS),)),
        ],
        compiler_params=pltpu.CompilerParams(
            vmem_limit_bytes=100 * 1024 * 1024,
            disable_semaphore_checks=True,
        ),
    )(
        A_x.reshape(1, M),
        A_c_kv.reshape(sk, DC),
        A_w_q.reshape(M * H, D),
        A_w_uk.reshape(DC * H, D),
        A_w_uv.reshape(DC * H, D),
        A_w_o.reshape(H * D, M),
        B_w1.T,
        B_w2,
    )
    return out.reshape(1, 1, M)
```
